```python
import os as _os
_os.environ.setdefault("JAX_PLATFORMS", "cpu")
import jax
import jax.numpy as jnp

def _softmax(x, axis=-1):
    return jax.nn.softmax(x, axis=axis)
def _gelu(x):
    return jax.nn.gelu(x, approximate=True)
def _silu(x):
    return jax.nn.silu(x)
def _sigmoid(x):
    return jax.nn.sigmoid(x)
def _layernorm(x, axis=-1, eps=1e-5):
    m = jnp.mean(x, axis=axis, keepdims=True)
    v = jnp.var(x, axis=axis, keepdims=True)
    return (x - m) / jnp.sqrt(v + eps)
def _scatter_add(tgt, idx, src, axis=0):
    return tgt.at[idx].add(src)
def _segment_sum(src, seg, n):
    return jax.ops.segment_sum(src, seg, n)
class _Rng:
    def __init__(self, key):
        self._k = key
    def _next(self):
        self._k, sub = jax.random.split(self._k)
        return sub
    def normal(self, shape):
        return jax.random.normal(self._next(), shape, dtype=jnp.bfloat16)
    def randint(self, lo, hi, shape):
        return jax.random.randint(self._next(), shape, lo, hi, dtype=jnp.int32)
    def uniform(self, shape, lo=0.0, hi=1.0):
        return jax.random.uniform(self._next(), shape, jnp.bfloat16, lo, hi)
    def permutation(self, n):
        return jax.random.permutation(self._next(), n)


kernel_name = 'concat_heads__ssm_conv_h3__sliding_block__prompt'

def setup_inputs():
    _rng = _Rng(jax.random.key(int.from_bytes(__import__("os").urandom(4), "little")))
    _w = (lambda a: (lambda t: t.astype(jnp.bfloat16) if jnp.issubdtype(t.dtype, jnp.floating) else t)(jnp.asarray(a)))
    def _A_setup():
        B, S, D = 1, 2048, 512
        ks = 4
        return {
            "q": _w((lambda *s: _rng.normal(s) * 0.05)(B, S, D)),
            "k": _w((lambda *s: _rng.normal(s) * 0.2)(B, S, D)),
            "v": _w((lambda *s: _rng.normal(s) * 0.2)(B, S, D)),
            "shift_k": _w((lambda *s: _rng.normal(s) * 0.2)(D, ks) * 0.5),
            "ssm_k": _w((lambda *s: _rng.normal(s) * 0.2)(D, S) * (1.0 / S ** 0.5)),
            "ssm_D": _w((lambda *s: _rng.normal(s) * 0.2)(D)),
        }
    _A_in = _A_setup()

    def _B_setup():
        B, S, D = 1, 2048, 512
        return {
            "x": _w((lambda *s: _rng.normal(s) * 0.2)(B, S, D)),
            "wqkv": _w((lambda *s: _rng.normal(s) * 0.2)(D, 3 * D)),
            "wo": _w((lambda *s: _rng.normal(s) * 0.05)(D, D)),
        }
    _B_in = _B_setup()

    return {
        "A_q": _A_in["q"],
        "A_k": _A_in["k"],
        "A_v": _A_in["v"],
        "A_shift_k": _A_in["shift_k"],
        "A_ssm_k": _A_in["ssm_k"],
        "A_ssm_D": _A_in["ssm_D"],
        "B_x": _B_in["x"],
        "B_wqkv": _B_in["wqkv"],
        "B_wo": _B_in["wo"],
    }

def reference(A_q, A_k, A_v, A_shift_k, A_ssm_k, A_ssm_D, B_x, B_wqkv, B_wo):
    def _A_ref(q, k, v, shift_k, ssm_k, ssm_D):
        B, S, D = q.shape
        ks = shift_k.shape[-1]
        k_pad = jnp.pad(k, ((0, 0), (ks - 1, 0), (0, 0)))
        k_shift = jnp.zeros_like(k)
        for t in range(ks):
            k_shift = k_shift + k_pad[:, t:t + S, :] * shift_k[:, ks - 1 - t][None, None, :]
        kv = k_shift * v
        L = 2 * S
        kv_pad = jnp.pad(kv, ((0, 0), (0, S), (0, 0)))
        kf_pad = jnp.pad(ssm_k, ((0, 0), (0, S)))
        kv_f = (lambda x, axes=(-2,-1): jnp.fft.rfft2(x.astype(jnp.float32), axes=axes))(kv_pad[:, None, :, :], axes=(1, 2))
        kf_f = (lambda x, axes=(-2,-1): jnp.fft.rfft2(x.astype(jnp.float32), axes=axes))(kf_pad[:, None, :], axes=(1, 2))
        kf_f = (lambda x, *d: x.transpose(*d))(kf_f, 1, 2, 0)
        y_f = kv_f * kf_f[None, :, :, :]
        y = (lambda x, s, axes=(-2,-1): jnp.fft.irfft2(x, s=s, axes=axes).astype(jnp.bfloat16))(y_f, (1, L), axes=(1, 2))[:, 0, :S, :]
        y = y + kv * ssm_D[None, None, :]
        return q * y

    def _B_ref(x, wqkv, wo):
        B, S, D = x.shape
        H = 32; Dh = D // H; W = 256
        qkv = (lambda x, *d: x.transpose(*d))((x @ wqkv).reshape(B, S, 3, H, Dh), 2, 0, 3, 1, 4)
        q, k, v = qkv[0], qkv[1], qkv[2]
        scores = jnp.einsum("bhqd,bhkd->bhqk", q, k) * (Dh ** -0.5)
        idx = jnp.arange(S)
        mask = (idx[:, None] - idx[None, :] >= 0) & (idx[:, None] - idx[None, :] < W)
        scores = jnp.where(mask[None, None], scores, -1e9)
        p = _softmax(scores, axis=-1)
        o = jnp.einsum("bhqk,bhkd->bhqd", p, v)
        return (lambda x, *d: x.transpose(*d))(o, 0, 2, 1, 3).reshape(B, S, D) @ wo

    a = _A_ref(A_q, A_k, A_v, A_shift_k, A_ssm_k, A_ssm_D)
    b = _B_ref(B_x, B_wqkv, B_wo)
    return jnp.concatenate([a, b], axis=-1)
```

```python
import functools, math
import numpy as np
import jax
import jax.numpy as jnp
import jax.experimental.pallas as pl
import jax.experimental.pallas.tpu as pltpu

S = 2048; D = 512; NH = 32; DH = 16; WIN = 256
C = 128; NC = S // C
BF = jnp.bfloat16; F32 = jnp.float32; U32 = jnp.uint32
QSCALE = (DH ** -0.5) * math.log2(math.e)
NEG = -1e30

def _dft_mats():
    n = np.arange(C)
    k = np.concatenate([np.arange(0, C, 2), np.arange(1, C, 2)])
    th = 2 * np.pi * np.outer(k + 0.5, n) / (2 * C)
    ff = np.concatenate([np.cos(th), -np.sin(th)], 0)
    fi0 = ff.T / C
    cols = []
    for w in range(C // 8):
        for r in range(8):
            cols += [8 * w + r, C + 8 * w + r]
    fi = fi0[:, np.array(cols)]
    return ff.astype(np.float32), fi.astype(np.float32)

def _nt(a, b):
    return jax.lax.dot_general(a, b, (((1,), (1,)), ((), ())), preferred_element_type=F32)

def _tn(a, b):
    return jax.lax.dot_general(a, b, (((0,), (0,)), ((), ())), preferred_element_type=F32)

def _nn(a, b):
    return jnp.dot(a, b, preferred_element_type=F32)

def _pk(x):
    return pltpu.bitcast(x.astype(BF), U32)

def _upk(x):
    return pltpu.bitcast(x, BF)

def _mo(x, m):
    return x if isinstance(x, int) else pl.multiple_of(x, m)


def kernel(q_hbm, k_hbm, v_hbm, sh_ref, h_hbm, d_ref, x_hbm, wqkv_hbm, wo_hbm, ff_ref, fi_ref,
           o_hbm,
           wqvT, wkp, kbuf, vtbuf, qbd, ot, sbuf, kpad, uh, hprev, ybuf, kvbuf, cst, zs,
           q_ref, v_ref, h_ref, x_ref, wqkv_ref, wo_ref, o_ref, sems, osem):
    cnt = [0]
    def mk(src, dst):
        c = pltpu.make_async_copy(src, dst, sems.at[cnt[0]])
        cnt[0] += 1
        return c
    def w_cp(i):
        return mk(wqkv_hbm.at[:, i * D:(i + 1) * D], wqkv_ref.at[:, i * D:(i + 1) * D])
    def x_cp(r0, r1):
        return mk(x_hbm.at[r0:r1, :], x_ref.at[r0:r1, :])
    def conv_cps(g):
        r0, r1 = 512 * g, 512 * (g + 1)
        return [mk(h_hbm.at[:, r0:r1], h_ref.at[:, r0:r1]),
                mk(k_hbm.at[r0:r1, :], kpad.at[16 + r0:16 + r1, :]),
                mk(v_hbm.at[r0:r1, :], v_ref.at[r0:r1, :])]
    cwq, cwv, cwk, cx0 = w_cp(0), w_cp(2), w_cp(1), x_cp(0, 256)
    S1 = conv_cps(0) + [mk(wo_hbm, wo_ref)]
    S2 = conv_cps(1) + [x_cp(256, 512)]
    S3 = conv_cps(2) + [x_cp(512, 768)]
    S4 = conv_cps(3) + [x_cp(768, 1024)]
    S5 = [x_cp(1024, 2048), mk(q_hbm, q_ref)]
    def start(l):
        for c in l: c.start()
    def wait(l):
        for c in l: c.wait()
    def out_cp(r0, c0):
        return pltpu.make_async_copy(o_ref.at[pl.ds(r0, 128), c0:c0 + D], o_hbm.at[pl.ds(r0, 128), c0:c0 + D], osem)

    start([cwq, cwv, cwk, cx0])
    eye = (jax.lax.broadcasted_iota(jnp.int32, (8, 4), 0) ==
           jax.lax.broadcasted_iota(jnp.int32, (8, 4), 1)).astype(BF)
    cst[0:8, :] = _nt(eye, sh_ref[...])
    cst[8:16, :] = jnp.broadcast_to(d_ref[...].astype(F32).reshape(1, D), (8, D))
    kpad[0:16, :] = jnp.zeros((16, D), BF)
    hprev[...] = jnp.zeros((2 * C, D), F32)
    for i in range(NC):
        zs[i] = 0
    cwq.wait()
    wqvT[0:D // 2, :] = _pk(wqkv_ref[:, 0:D].T)
    cwv.wait()
    start(S1)
    wqvT[D // 2:D, :] = _pk(wqkv_ref[:, 2 * D:3 * D].T)
    cwk.wait(); cx0.wait()
    wkp[...] = _pk(wqkv_ref[:, D:2 * D])

    lane16 = jax.lax.broadcasted_iota(jnp.int32, (16, 512), 1)
    row16 = jax.lax.broadcasted_iota(jnp.int32, (16, 512), 0)
    lo16 = jax.lax.broadcasted_iota(jnp.int32, (16, 128), 1) < 64

    def proj_k(a):
        r0 = _mo(a * 128, 128)
        xb = x_ref[pl.ds(r0, 128), :]
        kb = _nn(xb, _upk(wkp[...]))
        kbuf[pl.ds(_mo((WIN + r0) // 2, 64), 64), :] = _pk(kb)

    def proj_qv(a):
        r0 = _mo(a * 128, 128)
        slot = a % 2
        xb = x_ref[pl.ds(r0, 128), :]
        qvt = _nt(_upk(wqvT[...]), xb)
        vtbuf[:, pl.ds(WIN + r0, 128)] = _pk(qvt[D:2 * D])
        qt = qvt[0:D] * QSCALE
        qtr = pltpu.roll(qt, 64, 1)
        for h in range(NH):
            e = h % 2
            a0 = qt[16 * h:16 * h + 16]
            a1 = qtr[16 * h:16 * h + 16]
            if e == 0:
                p0 = jnp.where(lo16, a0, 0.0)
                p1 = jnp.where(lo16, a1, 0.0)
            else:
                p0 = jnp.where(lo16, 0.0, a1)
                p1 = jnp.where(lo16, 0.0, a0)
            qbd[slot, 0, 8 * h:8 * h + 8, :] = _pk(p0)
            qbd[slot, 1, 8 * h:8 * h + 8, :] = _pk(p1)

    def win_cfg(a, b):
        if isinstance(a, int) and a < 2:
            inval = WIN - (a * 128 + 64 * b)
            return False, max(64, inval)
        return True, 64

    def qk(a, n, fill=None):
        g, b = n // 2, n % 2
        has_head, ms = win_cfg(a, b)
        slot = a % 2
        base = _mo(a * 64 + 32 * b, 32)
        lanes = slice(128 * g, 128 * (g + 1))
        pieces = []
        for t in range(4):
            if has_head:
                pieces.append(kbuf[pl.ds(base + 8 * t, 8), lanes])
            pieces.append(kbuf[pl.ds(base + 128 + 8 * t, 8), lanes])
        nmid = 256 - ms
        if nmid:
            pieces.append(kbuf[pl.ds(base + ms // 2, nmid // 2), lanes])
        kwin = _upk(jnp.concatenate(pieces, 0))
        z = jnp.zeros((16, 128), U32)
        cols = []
        for pp in range(4):
            p = 4 * g + pp
            blk = [z] * 4
            blk[pp] = qbd[slot, b, 16 * p:16 * p + 16, :]
            cols.append(jnp.concatenate(blk, 0))
        wq = _upk(jnp.concatenate(cols, 1))
        s = _nn(kwin, wq)
        mx = None
        off = 0
        for t in range(4):
            tri = (row16 + 16 * t) <= (lane16 & 63)
            if has_head:
                hd = s[off:off + 16]; off += 16
            else:
                hd = NEG
            tl = s[off:off + 16]; off += 16
            ht = jnp.where(tri, tl, hd)
            sbuf[n % 2, 16 * t:16 * t + 16, :] = ht
            mx = ht if mx is None else jnp.maximum(mx, ht)
            if fill: fill(ht[0:8, 0:128])
        for t in range(nmid // 16):
            md = s[off:off + 16]; off += 16
            sbuf[n % 2, ms + 16 * t:ms + 16 * t + 16, :] = md
            mx = jnp.maximum(mx, md)
            if fill: fill(md[0:8, 0:128])
        return jnp.max(mx, axis=0, keepdims=True)

    def sm_pieces(a, n, m, st):
        g, b = n // 2, n % 2
        has_head, ms = win_cfg(a, b)
        st['hs'] = []; st['ts'] = []; st['mid'] = []; st['l'] = None
        def piece(t):
            sv = sbuf[n % 2, 32 * (t // 2):32 * (t // 2) + 32, :][16 * (t % 2):16 * (t % 2) + 16]
            p = jnp.exp2(sv - m)
            st['l'] = p if st['l'] is None else st['l'] + p
            if t < 4:
                tri = (row16 + 16 * t) <= (lane16 & 63)
                if has_head:
                    st['hs'].append(jnp.where(tri, 0.0, p))
                    st['ts'].append(jnp.where(tri, p, 0.0))
                else:
                    st['ts'].append(p)
            else:
                st['mid'].append(p)
        return [functools.partial(piece, t) for t in list(range(4)) + list(range(ms // 16, 16))]

    def pv(a, n, st):
        g, b = n // 2, n % 2
        has_head, ms = win_cfg(a, b)
        r0 = _mo(a * 128, 128)
        rinv = 1.0 / jnp.sum(st['l'], axis=0, keepdims=True)
        first = 64 * b + (0 if has_head else ms)
        t0 = first // 128
        parts = []
        if first > 128 * t0:
            parts.append(jnp.zeros((first - 128 * t0, 512), F32))
        parts += st['hs'] + st['mid'] + st['ts']
        if b == 0:
            parts.append(jnp.zeros((64, 512), F32))
        pw = jnp.concatenate(parts, 0)
        kk = 384 - 128 * t0
        rs = []
        for pp in range(4):
            p = 4 * g + pp
            vt = _upk(vtbuf[16 * p:16 * p + 16, pl.ds(r0 + 128 * t0, kk)])
            r = _nn(vt, pw[:, 128 * pp:128 * (pp + 1)].astype(BF)) * rinv[:, 128 * pp:128 * (pp + 1)]
            rs.append(r)
        return rs

    def finish(g, rs0, rs1):
        for pp in range(4):
            p = 4 * g + pp
            r0_, r1_ = rs0[pp], rs1[pp]
            r0r = pltpu.roll(r0_[16:32], 64, 1)
            r1r = pltpu.roll(r1_[0:16], 64, 1)
            oe = jnp.where(lo16, r0_[0:16], r1r)
            oo = jnp.where(lo16, r0r, r1_[16:32])
            ot[16 * p:16 * p + 16, :] = _pk(jnp.concatenate([oe, oo], 0))

    def outproj(a):
        r0 = _mo(a * 128, 128)
        ob = _tn(_upk(ot[...]), wo_ref[...])
        o_ref[pl.ds(r0, 128), D:2 * D] = ob.astype(BF)
        out_cp(r0, D).start()

    def attn_block(a, extras, fine=None, first=False, last=False):
        fine = fine or [[] for _ in range(9)]
        def mkfill(smp, fl):
            st = {'k': 0}
            nfl = len(fl)
            rel = {int(round((i + 0.3) * 16.0 / max(nfl, 1))): i for i in range(nfl)}
            def fill(tok):
                k = st['k']; st['k'] += 1
                if smp:
                    smp.pop(0)()
                if k in rel:
                    fl[rel[k]](tok)
            return fill
        m_next = qk(a, 0, mkfill([], fine[0]))
        if not first:
            outproj(a - 1)
        prev = None
        for n in range(8):
            m = m_next
            st = {}
            smp = sm_pieces(a, n, m, st)
            if n < 7:
                m_next = qk(a, n + 1, mkfill(smp, fine[n + 1]))
            elif not last:
                proj_k(a + 1)
            for f in smp: f()
            for f in extras[n]:
                f()
            rs = pv(a, n, st)
            if n % 2 == 0:
                prev = rs
            else:
                finish(n // 2, prev, rs)
        if not last:
            proj_qv(a + 1)

    def scatter(j, c0, arrs):
        for ci, arr in enumerate(arrs):
            for w in range(64):
                fg, c = w // 4, w % 4
                uh[w // 8, w % 8, (c0 + ci) * NC + j] = arr[8 * fg:8 * fg + 8, 128 * c:128 * (c + 1)]

    def fwd_h(j):
        r0 = _mo(j * C, C)
        hc = _nt(ff_ref[...], h_ref[:, pl.ds(r0, C)])
        hp = hprev[...]
        H2 = C // 2
        hre = jnp.concatenate([hc[0:H2] - hp[C:C + H2], hc[H2:C] + hp[C + H2:2 * C]], 0)
        him = jnp.concatenate([hc[C:C + H2] + hp[0:H2], hc[C + H2:2 * C] - hp[H2:C]], 0)
        scatter(j, 3, (hre, him - hre, hre + him))
        hprev[...] = hc

    def fwd_u(j):
        r0 = _mo(j * C, C)
        kk = kpad[pl.ds(r0, C + 16), :].astype(F32)
        ks = (kk[16:16 + C] * cst[0:1, :] + kk[15:15 + C] * cst[1:2, :]
              + kk[14:14 + C] * cst[2:3, :] + kk[13:13 + C] * cst[3:4, :])
        kv = (ks * v_ref[pl.ds(r0, C), :].astype(F32)).astype(BF)
        kvbuf[pl.ds(_mo(r0 // 2, 64), C // 2), :] = pltpu.bitcast(kv, U32)
        u = _nn(ff_ref[...], kv)
        ua = u[0:C]; ub = u[C:2 * C]
        scatter(j, 0, (ua, ub, ua + ub))

    def item_outs(blk, n, outs, zi):
        bz = blk + zs[zi]
        acc = {o: None for o in outs}
        for j in range(max(outs) + 1):
            ua = uh[bz, n, 0 * NC + j]; ub = uh[bz, n, 1 * NC + j]; us = uh[bz, n, 2 * NC + j]
            for o in outs:
                m = o - j
                if m < 0:
                    continue
                t1 = uh[bz, n, 3 * NC + m] * us
                t2 = uh[bz, n, 4 * NC + m] * ua
                t3 = uh[bz, n, 5 * NC + m] * ub
                if acc[o] is None:
                    acc[o] = (t1, t2, t3)
                else:
                    acc[o] = (acc[o][0] + t1, acc[o][1] + t2, acc[o][2] + t3)
        for o in outs:
            a1, a2, a3 = acc[o]
            ybuf[blk, n, o] = pltpu.pack_elementwise([a1 - a3, a1 + a2], packed_dtype=BF)

    PIECES = [(0, 1, 2, 3, 4, 5), (6, 7), (8, 9), (10, 11), (12, 13), (14, 15)]
    def item_pieces(blk, n):
        def pc(pi, tok):
            uh[blk + zs[15], n, 6 * NC] = tok
            item_outs(blk, n, PIECES[pi], pi)
        return [functools.partial(pc, pi) for pi in range(len(PIECES))]

    def inv(i):
        r0 = _mo(i * C, C)
        yy = jnp.concatenate(
            [jnp.concatenate([ybuf[(4 * fg + c) // 8, (4 * fg + c) % 8, i] for c in range(4)], 1)
             for fg in range(16)], 0)
        y = _nn(fi_ref[...], _upk(yy))
        kv = _upk(kvbuf[pl.ds(_mo(r0 // 2, 64), C // 2), :]).astype(F32)
        y = y + kv * cst[8:9, :]
        o_ref[pl.ds(r0, C), 0:D] = (q_ref[pl.ds(r0, C), :].astype(F32) * y).astype(BF)
        out_cp(r0, 0).start()

    P = functools.partial
    def fwd_extras(a):
        ex = [[] for _ in range(8)]
        for u in range(4):
            ex[2 * u].append(P(fwd_h, 4 * a + u))
            ex[2 * u + 1].append(P(fwd_u, 4 * a + u))
        return ex

    proj_k(0); proj_qv(0)
    def mid0():
        wait(S1); start(S2)
    ex0 = [[] for _ in range(8)]
    ex0[3].append(mid0)
    for u in range(4):
        ex0[4 + u] += [P(fwd_h, u), P(fwd_u, u)]
    with jax.named_scope('blk0'):
        attn_block(0, ex0, first=True)
    wait(S2); start(S3); start(S4)
    with jax.named_scope('blk1'):
        attn_block(1, fwd_extras(1))
    wait(S3); start(S5)
    with jax.named_scope('blk2'):
        attn_block(2, fwd_extras(2))
    wait(S4)
    with jax.named_scope('blk3'):
        attn_block(3, fwd_extras(3))
    wait(S5)

    def body_i(a, c):
        fine = [item_pieces(a - 4, n) for n in range(8)] + [[]]
        attn_block(a, [[] for n in range(8)], fine)
        return c
    with jax.named_scope('phI'):
        jax.lax.fori_loop(4, 12, body_i, 0)

    def inv_extras(a):
        ex = [[] for _ in range(8)]
        for u in range(4):
            ex[2 * u].append(P(inv, 4 * (a - 12) + u))
        return ex

    def body_v(a, c):
        attn_block(a, inv_extras(a))
        return c
    with jax.named_scope('phV'):
        jax.lax.fori_loop(12, 15, body_v, 0)
    with jax.named_scope('blk15'):
        attn_block(15, inv_extras(15), last=True)
        outproj(15)
    for _ in range(2 * NC):
        out_cp(0, 0).wait()


@jax.jit
def pallas_concat_heads__ssm_conv_h3__sliding_block__prompt_kernel(
        A_q, A_k, A_v, A_shift_k, A_ssm_k, A_ssm_D, B_x, B_wqkv, B_wo):
    ff, fi = _dft_mats()
    ff = jnp.asarray(ff, BF); fi = jnp.asarray(fi, BF)
    ANY = pl.BlockSpec(memory_space=pl.ANY)
    VM = pl.BlockSpec(memory_space=pltpu.VMEM)
    out = pl.pallas_call(
        kernel,
        out_shape=jax.ShapeDtypeStruct((S, 2 * D), BF),
        in_specs=[ANY, ANY, ANY, VM, ANY, VM, ANY, ANY, ANY, VM, VM],
        out_specs=ANY,
        scratch_shapes=[
            pltpu.VMEM((D, D), U32),
            pltpu.VMEM((D // 2, D), U32),
            pltpu.VMEM(((S + WIN) // 2, D), U32),
            pltpu.VMEM((D // 2, S + WIN), U32),
            pltpu.VMEM((2, 2, D // 2, 128), U32),
            pltpu.VMEM((D // 2, 128), U32),
            pltpu.VMEM((2, 256, 512), F32),
            pltpu.VMEM((S + 16, D), BF),
            pltpu.VMEM((8, 8, 6 * NC + 1, 8, 128), F32),
            pltpu.VMEM((2 * C, D), F32),
            pltpu.VMEM((8, 8, NC, 8, 128), U32),
            pltpu.VMEM((S // 2, D), U32),
            pltpu.VMEM((16, D), F32),
            pltpu.SMEM((NC,), jnp.int32),
            pltpu.VMEM((S, D), BF),
            pltpu.VMEM((S, D), BF),
            pltpu.VMEM((D, S), BF),
            pltpu.VMEM((S, D), BF),
            pltpu.VMEM((D, 3 * D), BF),
            pltpu.VMEM((D, D), BF),
            pltpu.VMEM((S, 2 * D), BF),
            pltpu.SemaphoreType.DMA((24,)),
            pltpu.SemaphoreType.DMA(()),
        ],
        compiler_params=pltpu.CompilerParams(vmem_limit_bytes=100 * 1024 * 1024),
    )(A_q.reshape(S, D), A_k.reshape(S, D), A_v.reshape(S, D), A_shift_k, A_ssm_k, A_ssm_D,
      B_x.reshape(S, D), B_wqkv, B_wo, ff, fi)
    return out.reshape(1, S, 2 * D)
```

```python
import functools
import math

import numpy as np
import jax
import jax.numpy as jnp
import jax.experimental.pallas as pl
import jax.experimental.pallas.tpu as pltpu

S = 2048
D = 512
NH = 32
DH = 16
WIN = 256
C = 128
NC = S // C
BF = jnp.bfloat16
F32 = jnp.float32
U32 = jnp.uint32
QSCALE = (DH ** -0.5) * math.log2(math.e)
NEG = -1e30
IPB = 12


def _dft_mats():
    n = np.arange(C)
    k = np.arange(C)
    th = 2 * np.pi * np.outer(k + 0.5, n) / (2 * C)
    sg = np.where(k % 2 == 0, 1.0, -1.0)[:, None]
    ff = np.concatenate([np.cos(th), -np.sin(th) * sg], 0)
    fi0 = ff.T / C
    cols = []
    for f in range(C):
        cols += [f, C + f]
    fi = fi0[:, np.array(cols)]
    return ff.astype(np.float32), fi.astype(np.float32)


def _nt(a, b):
    return jax.lax.dot_general(a, b, (((1,), (1,)), ((), ())), preferred_element_type=F32)


def _tn(a, b):
    return jax.lax.dot_general(a, b, (((0,), (0,)), ((), ())), preferred_element_type=F32)


def _nn(a, b):
    return jnp.dot(a, b, preferred_element_type=F32)


def _pk(x):
    return pltpu.bitcast(x.astype(BF), U32)


def _upk(x):
    return pltpu.bitcast(x, BF)


def _pe(p):
    return pltpu.pack_elementwise([p[0:8], p[8:16]], packed_dtype=BF)


def _ue(x, i):
    return pltpu.unpack_elementwise(x, index=i, packed_dtype=BF, unpacked_dtype=F32)


def _mo(x, m):
    return x if isinstance(x, int) else pl.multiple_of(x, m)


def _kernel(q_hbm, k_hbm, v_hbm, sh_hbm, h_hbm, d_hbm, x_hbm, wqkv_hbm, wo_hbm, ff_hbm, fi_hbm,
            o_hbm,
            wqvT, wkp, wop, kbuf, vtbuf, qbd, ot, sbuf, kpad, uh, ybuf, kvbuf, cst, zs,
            q_ref, v_ref, h_ref, x_ref, wqkv_ref, wo_ref, o_ref, sh_ref, d_ref, ff_ref, fi_ref,
            sems, osem):
    P = functools.partial

    cnt = [0]

    def mk(src, dst):
        c = pltpu.make_async_copy(src, dst, sems.at[cnt[0]])
        cnt[0] += 1
        return c

    def w_cp(i):
        return mk(wqkv_hbm.at[:, i * D:(i + 1) * D], wqkv_ref.at[:, i * D:(i + 1) * D])

    def x_cp(r0, r1):
        return mk(x_hbm.at[r0:r1, :], x_ref.at[r0:r1, :])

    def conv_cps(g):
        r0, r1 = 512 * g, 512 * (g + 1)
        return [mk(h_hbm.at[:, r0:r1], h_ref.at[:, r0:r1]),
                mk(k_hbm.at[r0:r1, :], kpad.at[16 + r0:16 + r1, :]),
                mk(v_hbm.at[r0:r1, :], v_ref.at[r0:r1, :])]

    cx0, cwk, cwq, cwv, cx1 = x_cp(0, 128), w_cp(1), w_cp(0), w_cp(2), x_cp(128, 256)
    S1a = [mk(wo_hbm, wo_ref), x_cp(256, 384)]
    S1 = ([mk(sh_hbm, sh_ref), mk(d_hbm, d_ref), mk(ff_hbm, ff_ref), mk(fi_hbm, fi_ref)]
          + conv_cps(0))
    S2 = conv_cps(1) + [x_cp(384, 512)]
    S3 = conv_cps(2) + [x_cp(512, 768)]
    S4 = conv_cps(3)
    S5 = [x_cp(768, 2048), mk(q_hbm, q_ref)]

    def wait(copies):
        for c in copies:
            c.wait()

    def out_cp(r0, c0):
        return pltpu.make_async_copy(o_ref.at[pl.ds(r0, 128), c0:c0 + D],
                                     o_hbm.at[pl.ds(r0, 128), c0:c0 + D], osem)

    for c in [cx0, cwq, cwk, cwv, cx1] + S1a + S1 + S2 + S3 + S4 + S5:
        c.start()

    kpad[0:16, :] = jnp.zeros((16, D), BF)
    for i in range(NC):
        zs[i] = 0

    lane16 = jax.lax.broadcasted_iota(jnp.int32, (16, 512), 1)
    row16 = jax.lax.broadcasted_iota(jnp.int32, (16, 512), 0)
    lo16 = jax.lax.broadcasted_iota(jnp.int32, (16, 128), 1) < 64

    def wt_prep(col0, row0, rot):
        rr = jax.lax.broadcasted_iota(jnp.int32, (128, 128), 0)
        cc = jax.lax.broadcasted_iota(jnp.int32, (128, 128), 1)
        lo = rr & 15
        src = (rr & ~15) | (((lo << rot) | (lo >> (4 - rot))) & 15)
        pm = jnp.where(cc == src, 1.0, 0.0).astype(BF)
        for c in range(4):
            t = _nt(pm, wqkv_ref[:, col0 + 128 * c:col0 + 128 * (c + 1)])
            for g in range(8):
                wqvT[row0 + 64 * c + 8 * g:row0 + 64 * c + 8 * g + 8, :] = _pe(t[16 * g:16 * g + 16])

    def notick(tok):
        pass

    def proj_k(a, tick=notick):
        r0 = _mo(a * 128, 128)
        xb = x_ref[pl.ds(r0, 128), :]
        kr = _mo((WIN + r0) // 2, 64)
        for c in range(4):
            lanes = slice(128 * c, 128 * (c + 1))
            kb = _nn(xb, _upk(wkp[:, lanes]))
            for t in range(8):
                kbuf[pl.ds(kr + 8 * t, 8), lanes] = _pk(kb[16 * t:16 * t + 16])
                tick(kb[16 * t:16 * t + 8])

    def proj_q(a, tick=notick):
        r0 = _mo(a * 128, 128)
        slot = a % 2
        xb = x_ref[pl.ds(r0, 128), :]
        qt = _nt(_upk(wqvT[0:D // 2, :]), xb) * QSCALE
        qtr = pltpu.roll(qt, 64, 1)
        for h in range(NH):
            a0 = qt[16 * h:16 * h + 16]
            a1 = qtr[16 * h:16 * h + 16]
            if h % 2 == 0:
                p0 = jnp.where(lo16, a0, 0.0)
                p1 = jnp.where(lo16, a1, 0.0)
            else:
                p0 = jnp.where(lo16, 0.0, a1)
                p1 = jnp.where(lo16, 0.0, a0)
            qbd[slot, 0, 8 * h:8 * h + 8, :] = _pe(p0)
            qbd[slot, 1, 8 * h:8 * h + 8, :] = _pe(p1)
            tick(a0[0:8])

    def proj_v(a, tick=notick):
        r0 = _mo(a * 128, 128)
        xb = x_ref[pl.ds(r0, 128), :]
        vt_ = _nt(_upk(wqvT[D // 2:D, :]), xb)
        for t in range(NH):
            vtbuf[8 * t:8 * t + 8, pl.ds(WIN + r0, 128)] = _pe(vt_[16 * t:16 * t + 16])
            tick(vt_[16 * t:16 * t + 8])

    def win_cfg(a, b):
        if isinstance(a, int) and a < 2:
            inval = WIN - (a * 128 + 64 * b)
            return False, max(64, inval)
        return True, 64

    def qk(a, n, fill=None):
        g, b = n // 2, n % 2
        has_head, ms = win_cfg(a, b)
        slot = a % 2
        base = _mo(a * 64 + 32 * b, 32)
        lanes = slice(128 * g, 128 * (g + 1))
        pieces = []
        for t in range(4):
            if has_head:
                pieces.append(kbuf[pl.ds(base + 8 * t, 8), lanes])
            pieces.append(kbuf[pl.ds(base + 128 + 8 * t, 8), lanes])
        nmid = 256 - ms
        if nmid:
            pieces.append(kbuf[pl.ds(base + ms // 2, nmid // 2), lanes])
        kwin = _upk(jnp.concatenate(pieces, 0))
        z = jnp.zeros((16, 128), U32)
        cols = []
        for pp in range(4):
            p = 4 * g + pp
            blk = [z] * 4
            blk[pp] = qbd[slot, b, 16 * p:16 * p + 16, :]
            cols.append(jnp.concatenate(blk, 0))
        wq = _upk(jnp.concatenate(cols, 1))
        s = _nn(kwin, wq)
        mx = None
        off = 0
        for t in range(4):
            tri = (row16 + 16 * t) <= (lane16 & 63)
            if has_head:
                hd = s[off:off + 16]
                off += 16
            else:
                hd = NEG
            tl = s[off:off + 16]
            off += 16
            ht = jnp.where(tri, tl, hd)
            sbuf[n % 2, 16 * t:16 * t + 16, :] = ht
            mx = ht if mx is None else jnp.maximum(mx, ht)
            if fill:
                fill()
        for t in range(nmid // 16):
            md = s[off:off + 16]
            off += 16
            sbuf[n % 2, ms + 16 * t:ms + 16 * t + 16, :] = md
            mx = jnp.maximum(mx, md)
            if fill:
                fill()
        return jnp.max(mx, axis=0, keepdims=True)

    def sm_pieces(a, n, m, st):
        b = n % 2
        has_head, ms = win_cfg(a, b)
        st['hs'] = []
        st['ts'] = []
        st['mid'] = []
        st['l'] = None

        def piece(t):
            sv = sbuf[n % 2, 32 * (t // 2):32 * (t // 2) + 32, :][16 * (t % 2):16 * (t % 2) + 16]
            p = jnp.exp2(sv - m)
            st['l'] = p if st['l'] is None else st['l'] + p
            if t < 4:
                tri = (row16 + 16 * t) <= (lane16 & 63)
                if has_head:
                    st['hs'].append(jnp.where(tri, 0.0, p))
                    st['ts'].append(jnp.where(tri, p, 0.0))
                else:
                    st['ts'].append(p)
            else:
                st['mid'].append(p)
        return [P(piece, t) for t in list(range(4)) + list(range(ms // 16, 16))]

    def pv(a, n, st):
        g, b = n // 2, n % 2
        has_head, ms = win_cfg(a, b)
        r0 = _mo(a * 128, 128)
        rinv = 1.0 / jnp.sum(st['l'], axis=0, keepdims=True)
        first = 64 * b + (0 if has_head else ms)
        t0 = first // 128
        parts = []
        if first > 128 * t0:
            parts.append(jnp.zeros((first - 128 * t0, 512), F32))
        parts += st['hs'] + st['mid'] + st['ts']
        if b == 0:
            parts.append(jnp.zeros((64, 512), F32))
        pw = jnp.concatenate(parts, 0)
        kk = 384 - 128 * t0
        rs = []
        for pp in range(4):
            p = 4 * g + pp
            lanes = slice(128 * pp, 128 * (pp + 1))
            vt = _upk(vtbuf[16 * p:16 * p + 16, pl.ds(r0 + 128 * t0, kk)])
            rs.append(_nn(vt, pw[:, lanes].astype(BF)) * rinv[:, lanes])
        return rs

    def finish(g, rs0, rs1):
        for pp in range(4):
            p = 4 * g + pp
            r0_, r1_ = rs0[pp], rs1[pp]
            r0r = pltpu.roll(r0_[16:32], 64, 1)
            r1r = pltpu.roll(r1_[0:16], 64, 1)
            ot[16 * p:16 * p + 8, :] = _pe(jnp.where(lo16, r0_[0:16], r1r))
            ot[16 * p + 8:16 * p + 16, :] = _pe(jnp.where(lo16, r0r, r1_[16:32]))

    def outproj(a, tick=notick):
        r0 = _mo(a * 128, 128)
        for c in range(4):
            ob = _tn(_upk(ot[...]), _upk(wop[:, 128 * c:128 * (c + 1)]))
            for t in range(8):
                o_ref[pl.ds(r0 + 16 * t, 16), D + 128 * c:D + 128 * (c + 1)] = (
                    ob[16 * t:16 * t + 16].astype(BF))
                tick(ob[16 * t:16 * t + 8])
        out_cp(r0, D).start()

    def attn_block(a, extras, tick=notick, first=False, last=False):
        def mkfill(smp):
            def fill():
                if smp:
                    smp.pop(0)()
            return fill
        m_next = qk(a, 0)
        if not first:
            outproj(a - 1, tick)
            tick(None)
        prev = None
        for n in range(8):
            m = m_next
            st = {}
            smp = sm_pieces(a, n, m, st)
            if n < 7:
                m_next = qk(a, n + 1, mkfill(smp))
            elif not last:
                proj_k(a + 1, tick)
            for f in smp:
                f()
            for f in extras[n]:
                f()
            if n == 7 and not last:
                proj_q(a + 1, tick)
            rs = pv(a, n, st)
            if n % 2 == 0:
                prev = rs
            else:
                finish(n // 2, prev, rs)
        if not last:
            proj_v(a + 1, tick)

    def scatter(j, c0, arrs):
        for ci, arr in enumerate(arrs):
            for w in range(64):
                fg, c = w // 4, w % 4
                uh[w // IPB, w % IPB, c0 + 3 * j + ci] = arr[8 * fg:8 * fg + 8, 128 * c:128 * (c + 1)]

    def fwd_h(j):
        hc = _nt(ff_ref[...], h_ref[:, j * C:(j + 1) * C])
        hre = hc[0:C]
        him = hc[C:2 * C]
        scatter(j, 3 * NC, (hre, him - hre, hre + him))

    def fwd_u(j):
        u = _nn(ff_ref[...], _upk(kvbuf[64 * j:64 * (j + 1), :]))
        ua = u[0:C]
        ub = u[C:2 * C]
        scatter(j, 0, (ua, ub, ua + ub))

    def kv_gen(js):
        z = pl.multiple_of(zs[1] * 16, 16)
        row8 = jax.lax.broadcasted_iota(jnp.int32, (8, 128), 0)
        for j in js:
            for c in range(4):
                lanes = slice(128 * c, 128 * (c + 1))
                p1 = p2 = None
                for t in range(8):
                    r = j * C + 16 * t
                    if p1 is None:
                        xp = pltpu.bitcast(kpad[pl.ds(z + r, 16), lanes], U32)
                        p1 = pltpu.roll(xp, 1, 0)
                        p2 = pltpu.roll(xp, 2, 0)
                    x = pltpu.bitcast(kpad[pl.ds(z + (r + 16), 16), lanes], U32)
                    r1 = pltpu.roll(x, 1, 0)
                    r2 = pltpu.roll(x, 2, 0)
                    xm1 = jnp.where(row8 >= 1, r1, p1)
                    xm2 = jnp.where(row8 >= 2, r2, p2)
                    p1, p2 = r1, r2
                    e0 = _ue(x, 0)
                    o0 = _ue(x, 1)
                    e1 = _ue(xm1, 0)
                    o1 = _ue(xm1, 1)
                    o2 = _ue(xm2, 1)
                    s0 = cst[0:1, lanes]
                    s1 = cst[1:2, lanes]
                    s2 = cst[2:3, lanes]
                    s3 = cst[3:4, lanes]
                    kse = e0 * s0 + o1 * s1 + e1 * s2 + o2 * s3
                    kso = o0 * s0 + e0 * s1 + o1 * s2 + e1 * s3
                    vp = pltpu.bitcast(v_ref[r:r + 16, lanes], U32)
                    kvbuf[r // 2:r // 2 + 8, lanes] = pltpu.pack_elementwise(
                        [kse * _ue(vp, 0), kso * _ue(vp, 1)], packed_dtype=BF)
                    yield

    def mk_kv_tick(js, per, skip=0):
        gen = kv_gen(js)
        st = {'credit': 0.0, 'done': False, 'skip': skip}

        def tick(tok):
            if st['done'] or tok is None:
                return
            if st['skip'] > 0:
                st['skip'] -= 1
                return
            st['credit'] += per
            if st['credit'] < 1:
                return
            kpad[pl.ds(pl.multiple_of(S + 16 + zs[14] * 16, 16), 8), 0:128] = tok.astype(BF)
            while st['credit'] >= 1:
                st['credit'] -= 1
                try:
                    next(gen)
                except StopIteration:
                    st['done'] = True
                    return

        def flush():
            for _ in gen:
                pass
        return tick, flush

    def item_gen(blk, ns):
        bz = blk + zs[0]

        def ld(i):
            return (uh[bz, n, i], uh[bz, n, i + 1], uh[bz, n, i + 2])
        for n in ns:
            yprev = None
            for o in range(0, NC, 2):
                acc0 = acc1 = None
                hnext = None
                for j in range(o + 2):
                    ua, ub, us = ld(3 * j)
                    if hnext is None:
                        hnext = ld(3 * NC + 3 * (o + 1 - j))
                    t = (hnext[0] * us, hnext[1] * ua, hnext[2] * ub)
                    acc1 = t if acc1 is None else tuple(x + y for x, y in zip(acc1, t))
                    npairs = 1
                    if o - j >= 0:
                        hnext = ld(3 * NC + 3 * (o - j))
                        t = (hnext[0] * us, hnext[1] * ua, hnext[2] * ub)
                        acc0 = t if acc0 is None else tuple(x + y for x, y in zip(acc0, t))
                        npairs = 2
                    if j == o + 1:
                        for oo, acc in ((o, acc0), (o + 1, acc1)):
                            yr = acc[0] - acc[2]
                            yi = acc[0] + acc[1]
                            if yprev is None:
                                zr, zi = yr, yi
                            else:
                                zr = yr - yprev[1]
                                zi = yi + yprev[0]
                            yprev = (yr, yi)
                            ybuf[blk, n, oo] = pltpu.pack_elementwise([zr, zi], packed_dtype=BF)
                    yield (npairs, j == o + 1)

    def mk_tick(blk, ns, wgt, skip=0):
        gen = item_gen(blk, ns)
        st = {'credit': 0, 'done': False, 'bound': True, 'skip': skip}

        def tick(tok):
            if st['done']:
                return
            if tok is None:
                while not st['bound']:
                    try:
                        _, st['bound'] = next(gen)
                    except StopIteration:
                        st['done'] = True
                        return
                st['credit'] = 0
                return
            if st['skip'] > 0:
                st['skip'] -= 1
                return
            st['credit'] += wgt
            if st['credit'] < 2:
                return
            uh[blk + zs[15], 0, 6 * NC] = tok
            while st['credit'] >= 2:
                try:
                    k, st['bound'] = next(gen)
                    st['credit'] -= k
                except StopIteration:
                    st['done'] = True
                    return

        def flush():
            for _ in gen:
                pass
        return tick, flush

    def inv(i):
        r0 = i * C
        yy = jnp.concatenate(
            [jnp.concatenate([ybuf[(4 * fg + c) // IPB, (4 * fg + c) % IPB, i] for c in range(4)], 1)
             for fg in range(16)], 0)
        y = _nn(fi_ref[...], _upk(yy))
        kv = _upk(kvbuf[r0 // 2:(r0 + C) // 2, :]).astype(F32)
        y = y + kv * cst[8:9, :]
        o_ref[r0:r0 + C, 0:D] = (q_ref[r0:r0 + C, :].astype(F32) * y).astype(BF)
        out_cp(r0, 0).start()

    def mk_extras(hs, us):
        ex = [[] for _ in range(8)]
        for j, sl in hs:
            ex[sl].append(P(fwd_h, j))
        for j, sl in us:
            ex[sl].append(P(fwd_u, j))
        return ex

    cx0.wait()
    cwq.wait()
    wt_prep(0, 0, 2)
    proj_q(0)
    cwk.wait()
    wkp[...] = _pk(wqkv_ref[:, D:2 * D])
    proj_k(0)

    def v0():
        cwv.wait()
        cx1.wait()
        wt_prep(2 * D, D // 2, 3)
        proj_v(0)
    NOEX = [[] for _ in range(8)]
    attn_block(0, [[v0]] + NOEX[1:], first=True)

    wait(S1a)
    wop[...] = _pk(wo_ref[...])

    def w1():
        wait(S1)
        cst[0:4, :] = sh_ref[...].astype(F32)
        cst[8:16, :] = jnp.broadcast_to(d_ref[...].astype(F32).reshape(1, D), (8, D))
    tick, flush = mk_kv_tick([0, 1, 2, 3], 128 / 96, skip=32)
    ex1 = mk_extras([(0, 3), (1, 4), (2, 5), (3, 6)], [])
    ex1[2].append(w1)
    attn_block(1, ex1, tick)
    flush()

    wait(S2)
    tick, flush = mk_kv_tick(list(range(4, 8)), 1.0)
    attn_block(2, mk_extras([(4, 0), (5, 2), (6, 4), (7, 6)],
                            [(0, 1), (1, 3), (2, 5), (3, 7)]), tick)
    flush()

    wait(S3)
    wait(S4)
    tick, flush = mk_kv_tick(list(range(8, 14)), 1.5)
    attn_block(3, mk_extras([(8 + u, u) for u in range(8)],
                            [(4, 1), (5, 3), (6, 5), (7, 7)]), tick)
    flush()

    tick1, flush1 = mk_kv_tick([14, 15], 2.0)
    tick2, flush2 = mk_tick(5, range(4), 4 * 138 / 96, skip=32)

    def tick4(tok):
        tick1(tok)
        tick2(tok)
    ex4 = mk_extras([], [(8, 0), (9, 1), (10, 2), (11, 3), (12, 4), (13, 5), (14, 6), (15, 6)])
    ex4[0].insert(0, flush1)
    attn_block(4, ex4, tick4)
    flush2()

    wait(S5)

    def body_i(it, carry):
        tick_i, flush_i = mk_tick(it, range(IPB), 6 * 138 / 128)
        attn_block(5 + 2 * it, NOEX, tick_i)
        attn_block(6 + 2 * it, NOEX, tick_i)
        flush_i()
        return carry
    jax.lax.fori_loop(0, 5, body_i, 0)

    attn_block(15, [[P(inv, 2 * n), P(inv, 2 * n + 1)] for n in range(7)] + [[]], last=True)
    inv(14)
    outproj(15)
    inv(15)
    for _ in range(2 * NC):
        out_cp(0, 0).wait()


@jax.jit
def pallas_concat_heads__ssm_conv_h3__sliding_block__prompt_kernel(
        A_q, A_k, A_v, A_shift_k, A_ssm_k, A_ssm_D, B_x, B_wqkv, B_wo):
    ff, fi = _dft_mats()
    ff = jnp.asarray(ff, BF)
    fi = jnp.asarray(fi, BF)
    any_spec = pl.BlockSpec(memory_space=pl.ANY)
    out = pl.pallas_call(
        _kernel,
        out_shape=jax.ShapeDtypeStruct((S, 2 * D), BF),
        in_specs=[any_spec] * 11,
        out_specs=any_spec,
        scratch_shapes=[
            pltpu.VMEM((D, D), U32),
            pltpu.VMEM((D // 2, D), U32),
            pltpu.VMEM((D // 2, D), U32),
            pltpu.VMEM(((S + WIN) // 2, D), U32),
            pltpu.VMEM((D // 2, S + WIN), U32),
            pltpu.VMEM((2, 2, D // 2, 128), U32),
            pltpu.VMEM((D // 2, 128), U32),
            pltpu.VMEM((2, 256, 512), F32),
            pltpu.VMEM((S + 32, D), BF),
            pltpu.VMEM((6, IPB, 6 * NC + 1, 8, 128), F32),
            pltpu.VMEM((6, IPB, NC, 8, 128), U32),
            pltpu.VMEM((S // 2, D), U32),
            pltpu.VMEM((16, D), F32),
            pltpu.SMEM((NC,), jnp.int32),
            pltpu.VMEM((S, D), BF),
            pltpu.VMEM((S, D), BF),
            pltpu.VMEM((D, S), BF),
            pltpu.VMEM((S, D), BF),
            pltpu.VMEM((D, 3 * D), BF),
            pltpu.VMEM((D, D), BF),
            pltpu.VMEM((S, 2 * D), BF),
            pltpu.VMEM((4, D), BF),
            pltpu.VMEM((D,), BF),
            pltpu.VMEM((2 * C, C), BF),
            pltpu.VMEM((C, 2 * C), BF),
            pltpu.SemaphoreType.DMA((32,)),
            pltpu.SemaphoreType.DMA(()),
        ],
        compiler_params=pltpu.CompilerParams(vmem_limit_bytes=100 * 1024 * 1024),
    )(A_q.reshape(S, D), A_k.reshape(S, D), A_v.reshape(S, D), A_shift_k.T, A_ssm_k, A_ssm_D,
      B_x.reshape(S, D), B_wqkv, B_wo, ff, fi)
    return out.reshape(1, S, 2 * D)
```
